```python
import os as _os
_os.environ.setdefault("JAX_PLATFORMS", "cpu")
import jax
import jax.numpy as jnp

def _softmax(x, axis=-1):
    return jax.nn.softmax(x, axis=axis)
def _gelu(x):
    return jax.nn.gelu(x, approximate=True)
def _silu(x):
    return jax.nn.silu(x)
def _sigmoid(x):
    return jax.nn.sigmoid(x)
def _layernorm(x, axis=-1, eps=1e-5):
    m = jnp.mean(x, axis=axis, keepdims=True)
    v = jnp.var(x, axis=axis, keepdims=True)
    return (x - m) / jnp.sqrt(v + eps)
def _scatter_add(tgt, idx, src, axis=0):
    return tgt.at[idx].add(src)
def _segment_sum(src, seg, n):
    return jax.ops.segment_sum(src, seg, n)
class _Rng:
    def __init__(self, key):
        self._k = key
    def _next(self):
        self._k, sub = jax.random.split(self._k)
        return sub
    def normal(self, shape):
        return jax.random.normal(self._next(), shape, dtype=jnp.bfloat16)
    def randint(self, lo, hi, shape):
        return jax.random.randint(self._next(), shape, lo, hi, dtype=jnp.int32)
    def uniform(self, shape, lo=0.0, hi=1.0):
        return jax.random.uniform(self._next(), shape, jnp.bfloat16, lo, hi)
    def permutation(self, n):
        return jax.random.permutation(self._next(), n)


kernel_name = 'gated_mix__sliding_block__dense_activation_silu__prompt'

def setup_inputs():
    _rng = _Rng(jax.random.key(int.from_bytes(__import__("os").urandom(4), "little")))
    _w = (lambda a: (lambda t: t.astype(jnp.bfloat16) if jnp.issubdtype(t.dtype, jnp.floating) else t)(jnp.asarray(a)))
    def _A_setup():
        B, S, D = 1, 2048, 640
        return {
            "x": _w((lambda *s: _rng.normal(s) * 0.05)(B, S, D)),
            "wqkv": _w((lambda *s: _rng.normal(s) * 0.4)(D, 3 * D)),
            "wo": _w((lambda *s: _rng.normal(s) * 0.05)(D, D)),
        }
    _A_in = _A_setup()

    def _B_setup():
        B, S, D, F = 1, 2048, 640, 1536
        return {
            "x": _w((lambda *s: _rng.normal(s) * 0.05)(B, S, D)),
            "w1": _w((lambda *s: _rng.normal(s) * 1.6)(D, F) * (D ** -0.5)),
            "w2": _w((lambda *s: _rng.normal(s) * 1.6)(F, D) * (F ** -0.5)),
        }
    _B_in = _B_setup()

    return {
        "A_x": _A_in["x"],
        "A_wqkv": _A_in["wqkv"],
        "A_wo": _A_in["wo"],
        "B_x": _B_in["x"],
        "B_w1": _B_in["w1"],
        "B_w2": _B_in["w2"],
        "gate_w": _w((lambda *s: _rng.normal(s) * 0.05)(640) * 16.0),
    }

def reference(A_x, A_wqkv, A_wo, B_x, B_w1, B_w2, gate_w):
    def _A_ref(x, wqkv, wo):
        B, S, D = x.shape
        H = 32; Dh = D // H; W = 256
        qkv = (lambda x, *d: x.transpose(*d))((x @ wqkv).reshape(B, S, 3, H, Dh), 2, 0, 3, 1, 4)
        q, k, v = qkv[0], qkv[1], qkv[2]
        scores = jnp.einsum("bhqd,bhkd->bhqk", q, k) * (Dh ** -0.5)
        idx = jnp.arange(S)
        mask = (idx[:, None] - idx[None, :] >= 0) & (idx[:, None] - idx[None, :] < W)
        scores = jnp.where(mask[None, None], scores, -1e9)
        p = _softmax(scores, axis=-1)
        o = jnp.einsum("bhqk,bhkd->bhqd", p, v)
        return (lambda x, *d: x.transpose(*d))(o, 0, 2, 1, 3).reshape(B, S, D) @ wo

    def _B_ref(x, w1, w2):
        h = jnp.einsum("bsd,df->bsf", x, w1)
        h = _silu(h)
        out = jnp.einsum("bsf,fd->bsd", h, w2)
        return out

    x = A_x
    g = _sigmoid((x * gate_w).sum(-1, keepdims=True))
    a = _A_ref(x, A_wqkv, A_wo)
    b = _B_ref(x, B_w1, B_w2)
    return g * a + (1 - g) * b
```

```python
import functools
import jax
import jax.numpy as jnp
import jax.experimental.pallas as pl
import jax.experimental.pallas.tpu as pltpu

S, D, H, DH, WIN, F = 2048, 640, 32, 20, 256, 1536
TQ = 256
NSUB = TQ // 128
NB = S // 128
NT = (((1,), (1,)), ((), ()))
LOG2E = 1.4426950408889634
NEG = -1e9

CH = [[h for h in range(H) if DH * h < 128 * (c + 1) and DH * (h + 1) > 128 * c] for c in range(5)]


def _kernel(x_ref, wqkv_hbm, wo_hbm, w1_hbm, w2_hbm, gw_ref, o_ref,
            wqT_scr, wvT_scr, k_scr, vT_scr, wqkv_ref, wo_ref, w1_ref, w2_ref, sems):
    i = pl.program_id(0)
    cp_qkv = pltpu.make_async_copy(wqkv_hbm, wqkv_ref, sems.at[0])
    cp_w1 = pltpu.make_async_copy(w1_hbm, w1_ref, sems.at[1])
    cp_w2 = pltpu.make_async_copy(w2_hbm, w2_ref, sems.at[2])
    cp_wo = pltpu.make_async_copy(wo_hbm, wo_ref, sems.at[3])

    @pl.when(i == 0)
    def _():
        cp_qkv.start()
        k_scr[0:WIN, :] = jnp.zeros((WIN, D), jnp.bfloat16)
        vT_scr[0:2] = jnp.zeros((2, D, 128), jnp.bfloat16)
        cp_qkv.wait()
        cp_w1.start()
        cp_w2.start()
        cp_wo.start()
        wqT_scr[...] = wqkv_ref[:, 0:D].T
        wvT_scr[...] = wqkv_ref[:, 2 * D:3 * D].T

    x = x_ref[...]
    k = jnp.dot(x, wqkv_ref[:, D:2 * D], preferred_element_type=jnp.float32)
    k_scr[pl.ds(pl.multiple_of(WIN + i * TQ, 128), TQ), :] = k.astype(jnp.bfloat16)
    qT = jax.lax.dot_general(wqT_scr[...], x, NT, preferred_element_type=jnp.float32)
    qT = qT * (DH ** -0.5 * LOG2E)
    vT = jax.lax.dot_general(wvT_scr[...], x, NT, preferred_element_type=jnp.float32)
    vT = vT.astype(jnp.bfloat16)
    for s in range(NSUB):
        vT_scr[2 + i * NSUB + s] = vT[:, s * 128:(s + 1) * 128]

    @pl.when(i == 0)
    def _():
        cp_w1.wait()
        cp_w2.wait()
        cp_wo.wait()

    row128 = jax.lax.broadcasted_iota(jnp.int32, (128, 128), 0)
    col128 = jax.lax.broadcasted_iota(jnp.int32, (128, 128), 1)
    row8 = jax.lax.broadcasted_iota(jnp.int32, (8, 128), 0)
    bias0 = jnp.where(row128 > col128, 0.0, NEG)
    bias2 = jnp.where(row128 <= col128, 0.0, NEG)

    carry = {}

    def stage_a(s, c):
        j = i * NSUB + s
        koff = pl.multiple_of(j * 128, 128)
        qc_blk = qT[c * 128:(c + 1) * 128, s * 128:(s + 1) * 128]
        ws = []
        for h in CH[c]:
            lo, hi = DH * h, DH * (h + 1)
            m = (row128 >= lo - c * 128) & (row128 < hi - c * 128)
            ws.append(jnp.where(m, qc_blk, 0.0).astype(jnp.bfloat16))
        w = jnp.concatenate(ws, axis=1)
        kc = k_scr[pl.ds(koff, 384), c * 128:(c + 1) * 128]
        sall = jnp.dot(kc, w, preferred_element_type=jnp.float32)
        out = []
        for n, h in enumerate(CH[c]):
            sT = sall[:, n * 128:(n + 1) * 128]
            if DH * (h + 1) > 128 * (c + 1):
                carry[s] = sT
                continue
            if DH * h < 128 * c:
                sT = sT + carry[s]
            s0 = sT[0:128] + bias0
            s1 = sT[128:256]
            s2 = sT[256:384] + bias2
            m0 = jnp.where(j >= 2, jnp.max(s0, axis=0, keepdims=True), NEG)
            m1 = jnp.where(j >= 1, jnp.max(s1, axis=0, keepdims=True), NEG)
            m2 = jnp.max(s2, axis=0, keepdims=True)
            mx = jnp.maximum(jnp.maximum(m0, m1), m2)
            out.append((h, s0, s1, s2, mx))
        return out

    res = {}

    def stage_b(s, items):
        j = i * NSUB + s
        for (h, s0, s1, s2, mx) in items:
            p0 = jnp.exp2(s0 - jnp.where(j >= 2, mx, -NEG))
            p1 = jnp.exp2(s1 - jnp.where(j >= 1, mx, -NEG))
            p2 = jnp.exp2(s2 - mx)
            l = (jnp.sum(p0, axis=0, keepdims=True) + jnp.sum(p1, axis=0, keepdims=True)
                 + jnp.sum(p2, axis=0, keepdims=True))
            pb = jnp.concatenate([p0, p1, p2], axis=0).astype(jnp.bfloat16)
            r0 = 80 * (h // 4) + 16 * (h % 4)
            vt = jnp.concatenate(
                [vT_scr[j + t, r0:r0 + 32, :] for t in range(3)], axis=1)
            oh = jnp.dot(vt, pb, preferred_element_type=jnp.float32)
            res[(s, h)] = oh * (1.0 / l)

    hs = []
    bs = []

    def ffn_piece(n):
        if n < 12:
            hh = jnp.dot(x, w1_ref[:, n * 128:(n + 1) * 128], preferred_element_type=jnp.float32)
            hh = 0.5 * hh
            hs.append((hh * (1.0 + jnp.tanh(hh))).astype(jnp.bfloat16))
        else:
            if len(hs) == 12:
                hs.append(jnp.concatenate(hs, axis=1))
            m = n - 12
            bs.append(jnp.dot(hs[12], w2_ref[:, m * 128:(m + 1) * 128], preferred_element_type=jnp.float32))

    stages = [(s, c) for s in range(NSUB) for c in range(5)]
    sched = [0, 1, 2, 3, 4, 5, 6, 7, 8, 9, 10, 11, None, 12, None, 13, None, 14, 15, 16]
    nxt = stage_a(*stages[0])
    for si, (s, c) in enumerate(stages):
        cur = nxt
        if si + 1 < len(stages):
            nxt = stage_a(*stages[si + 1])
        if sched[2 * si] is not None:
            ffn_piece(sched[2 * si])
        stage_b(s, cur[:3])
        if sched[2 * si + 1] is not None:
            ffn_piece(sched[2 * si + 1])
        stage_b(s, cur[3:])

    oT_subs = []
    for s in range(NSUB):
        groups = []
        for g in range(H // 4):
            h0, h1, h2, h3 = [res[(s, 4 * g + t)] for t in range(4)]
            groups.append(jnp.concatenate([
                h0[0:16],
                jnp.where(row8 < 4, h0[16:24], h1[0:8]),
                h1[8:24],
                h2[8:24],
                jnp.where(row8 < 4, h2[24:32], h3[8:16]),
                h3[16:32],
            ], axis=0))
        oT_subs.append(jnp.concatenate(groups, axis=0))
    oT = jnp.concatenate(oT_subs, axis=1)
    o = oT.T.astype(jnp.bfloat16)
    a = jnp.dot(o, wo_ref[...], preferred_element_type=jnp.float32)
    b = jnp.concatenate(bs, axis=1)

    z = jnp.sum(x.astype(jnp.float32) * gw_ref[...].astype(jnp.float32), axis=-1, keepdims=True)
    gt = jax.nn.sigmoid(z)
    o_ref[...] = (gt * a + (1.0 - gt) * b).astype(o_ref.dtype)


@jax.jit
def pallas_gated_mix__sliding_block__dense_activation_silu__prompt_kernel(
    A_x, A_wqkv, A_wo, B_x, B_w1, B_w2, gate_w):
    x = A_x.reshape(S, D)
    gw = gate_w.reshape(1, D)
    const = lambda i: (0, 0)
    out = pl.pallas_call(
        _kernel,
        grid=(S // TQ,),
        in_specs=[
            pl.BlockSpec((TQ, D), lambda i: (i, 0)),
            pl.BlockSpec(memory_space=pl.ANY),
            pl.BlockSpec(memory_space=pl.ANY),
            pl.BlockSpec(memory_space=pl.ANY),
            pl.BlockSpec(memory_space=pl.ANY),
            pl.BlockSpec((1, D), const),
        ],
        out_specs=pl.BlockSpec((TQ, D), lambda i: (i, 0)),
        out_shape=jax.ShapeDtypeStruct((S, D), jnp.bfloat16),
        scratch_shapes=[
            pltpu.VMEM((D, D), jnp.bfloat16),
            pltpu.VMEM((D, D), jnp.bfloat16),
            pltpu.VMEM((S + WIN, D), jnp.bfloat16),
            pltpu.VMEM((NB + 2, D, 128), jnp.bfloat16),
            pltpu.VMEM((D, 3 * D), jnp.bfloat16),
            pltpu.VMEM((D, D), jnp.bfloat16),
            pltpu.VMEM((D, F), jnp.bfloat16),
            pltpu.VMEM((F, D), jnp.bfloat16),
            pltpu.SemaphoreType.DMA((4,)),
        ],
        compiler_params=pltpu.CompilerParams(
            dimension_semantics=("arbitrary",),
            vmem_limit_bytes=100 * 2 ** 20),
    )(x, A_wqkv, A_wo, B_w1, B_w2, gw)
    return out.reshape(1, S, D)
```

```python
import functools
import jax
import jax.numpy as jnp
import jax.experimental.pallas as pl
import jax.experimental.pallas.tpu as pltpu

S, D, H, DH, WIN, F = 2048, 640, 32, 20, 256, 1536
TQ = 512
NSUB = TQ // 128
NST = S // TQ
NB = S // 128
NT = (((1,), (1,)), ((), ()))
LOG2E = 1.4426950408889634
NEG = -1e9

XOFF = {6: 0, 19: 20, 12: 40, 25: 60, 8: 80, 21: 100}
GLANE = 120
CH = [[(h, 128 * c, DH * h - 128 * c) for h in range(H)
       if (DH * h) // 128 == c and h not in XOFF] for c in range(5)]
CH.append([(h, DH * h - XOFF[h], XOFF[h]) for h in XOFF])
NCH = len(CH)
DK = 128 * NCH
KR = WIN + 64


def _kernel(x_hbm, wqkv_hbm, wo_hbm, w1_hbm, w2_hbm, gw_ref, o_ref,
            x_scr, z_scr, wT_scr, wk_scr, k_scr, qT_scr, vT_scr, wqv_ref, wo_ref, w1_ref, w2_ref, sems):
    i = pl.program_id(0)

    @pl.when(i == 0)
    def _():
        cp_x = [pltpu.make_async_copy(x_hbm.at[b * TQ:(b + 1) * TQ, :], x_scr.at[b * TQ:(b + 1) * TQ, :],
                                      sems.at[6 + b]) for b in range(NST)]
        cp_q = pltpu.make_async_copy(wqkv_hbm.at[:, 0:D], wqv_ref.at[0], sems.at[0])
        cp_k = pltpu.make_async_copy(wqkv_hbm.at[:, D:2 * D], wk_scr.at[:, 0:D], sems.at[1])
        cp_v = pltpu.make_async_copy(wqkv_hbm.at[:, 2 * D:3 * D], wqv_ref.at[1], sems.at[2])
        cp_w1 = pltpu.make_async_copy(w1_hbm, w1_ref, sems.at[3])
        cp_w2 = pltpu.make_async_copy(w2_hbm, w2_ref, sems.at[4])
        cp_wo = pltpu.make_async_copy(wo_hbm, wo_ref, sems.at[5])
        cp_k.start()
        cp_x[0].start()
        cp_x[1].start()
        cp_q.start()
        cp_x[2].start()
        cp_x[3].start()
        cp_v.start()
        cp_w1.start()
        cp_w2.start()
        cp_wo.start()
        k_scr[0:WIN, :] = jnp.zeros((WIN, DK), jnp.bfloat16)
        vT_scr[0:2] = jnp.zeros((2, D, 128), jnp.bfloat16)
        r = jax.lax.broadcasted_iota(jnp.int32, (D, 128), 0)
        c = jax.lax.broadcasted_iota(jnp.int32, (D, 128), 1)
        sel = None
        for h in XOFF:
            m = (r - DH * h == c - XOFF[h]) & (c >= XOFF[h]) & (c < XOFF[h] + DH)
            sel = m if sel is None else (sel | m)
        sel = jnp.where(sel, 1.0, 0.0).astype(jnp.bfloat16)
        gcol = jnp.broadcast_to(gw_ref[...].astype(jnp.float32).reshape(1, D), (128, D)).T
        cp_k.wait()
        wkx = jnp.dot(wk_scr[:, 0:D], sel, preferred_element_type=jnp.float32)
        wk_scr[:, D:DK] = jnp.where(c >= GLANE, gcol, wkx).astype(jnp.bfloat16)

        def xblk(b):
            return x_scr[pl.ds(pl.multiple_of(b * TQ, TQ), TQ), :]

        def kproj(b, carry):
            rows = pl.ds(pl.multiple_of(b * TQ, TQ), TQ)
            pltpu.make_async_copy(x_hbm.at[rows, :], x_scr.at[rows, :], sems.at[6 + b]).wait()
            k = jnp.dot(xblk(b), wk_scr[...], preferred_element_type=jnp.float32)
            k_scr[pl.ds(pl.multiple_of(WIN + b * TQ, 128), TQ), :] = k.astype(jnp.bfloat16)
            z_scr[rows, :] = k[:, D:DK]
            return carry
        jax.lax.fori_loop(0, NST - 1, kproj, 0)
        cp_q.wait()
        kproj(NST - 1, 0)
        wT_scr[...] = wqv_ref[0].T

        def qproj(b, carry):
            qT = jax.lax.dot_general(wT_scr[...], xblk(b), NT, preferred_element_type=jnp.float32)
            qT = qT * (DH ** -0.5 * LOG2E)
            for s in range(NSUB):
                qT_scr[b * NSUB + s] = qT[:, s * 128:(s + 1) * 128]
            return carry
        jax.lax.fori_loop(0, NST - 1, qproj, 0)
        cp_v.wait()
        qproj(NST - 1, 0)
        wqv_ref[0] = wqv_ref[1].T

        def vproj(b, carry):
            vT = jax.lax.dot_general(wqv_ref[0], xblk(b), NT,
                                     preferred_element_type=jnp.float32).astype(jnp.bfloat16)
            for s in range(NSUB):
                vT_scr[2 + b * NSUB + s] = vT[:, s * 128:(s + 1) * 128]
            return carry
        jax.lax.fori_loop(0, NST, vproj, 0)
        cp_w1.wait()
        cp_w2.wait()
        cp_wo.wait()

    x = x_scr[pl.ds(pl.multiple_of(i * TQ, TQ), TQ), :]

    row128 = jax.lax.broadcasted_iota(jnp.int32, (128, 128), 0)
    lo128 = jax.lax.broadcasted_iota(jnp.int32, (128, 128), 1) < 64
    row8 = jax.lax.broadcasted_iota(jnp.int32, (8, 128), 0)
    r64 = jax.lax.broadcasted_iota(jnp.int32, (64, 128), 0)
    c64 = jax.lax.broadcasted_iota(jnp.int32, (64, 128), 1) & 63
    bias_a = jnp.where(r64 > c64, 0.0, NEG)
    bias_d = jnp.where(r64 <= c64, 0.0, NEG)
    lo1 = jax.lax.broadcasted_iota(jnp.int32, (1, 128), 1) < 64
    lo64 = jax.lax.broadcasted_iota(jnp.int32, (64, 128), 1) < 64
    lo256 = jax.lax.broadcasted_iota(jnp.int32, (256, 128), 1) < 64

    def tree(op, v):
        n = v.shape[0]
        while n > 8:
            h = n // 2
            if h % 8:
                break
            v = op(v[0:h], v[h:n])
            n = h
        return v

    def colmax(v):
        return jnp.max(tree(jnp.maximum, v), axis=0, keepdims=True)

    def segmax(v0, v1, v2, j):
        m = jnp.maximum(jnp.maximum(jnp.where(j >= 2, tree(jnp.maximum, v0), NEG),
                                    jnp.where(j >= 1, tree(jnp.maximum, v1), NEG)),
                        tree(jnp.maximum, v2))
        return jnp.max(m, axis=0, keepdims=True)

    def colsum(v):
        return jnp.sum(tree(jnp.add, v), axis=0, keepdims=True)

    def stage_a(s, c):
        j = i * NSUB + s
        koff = pl.multiple_of(j * 128, 128)
        w1s, w2s = [], []
        heads = CH[c]
        for p in range(len(heads) // 2):
            (ha, ra, oa), (hb, rb, ob) = heads[2 * p], heads[2 * p + 1]
            qa = qT_scr[j, ra:ra + 128, :]
            qa = jnp.where((row128 >= oa) & (row128 < oa + DH), qa, 0.0)
            qb = qT_scr[j, rb:rb + 128, :]
            qb = jnp.where((row128 >= ob) & (row128 < ob + DH), qb, 0.0)
            qbr = pltpu.roll(qb, 64, 1)
            w1s.append(jnp.where(lo128, qa, qbr).astype(jnp.bfloat16))
            w2s.append(jnp.where(lo128, qbr, qa).astype(jnp.bfloat16))
        k1 = k_scr[pl.ds(koff, KR), c * 128:(c + 1) * 128]
        k2 = k_scr[pl.ds(koff + 64, KR), c * 128:(c + 1) * 128]
        s1all = jnp.dot(k1, jnp.concatenate(w1s, axis=1), preferred_element_type=jnp.float32)
        s2all = jnp.dot(k2, jnp.concatenate(w2s, axis=1), preferred_element_type=jnp.float32)
        out = []
        for p in range(len(heads) // 2):
            ha, hb = heads[2 * p][0], heads[2 * p + 1][0]
            t = s1all[:, p * 128:(p + 1) * 128]
            a0 = jnp.concatenate([t[0:64] + bias_a, t[64:128]], axis=0)
            a1 = t[128:256]
            a2 = t[256:KR] + bias_d
            mx1 = segmax(a0, a1, a2, j)
            t = s2all[:, p * 128:(p + 1) * 128]
            b0 = t[0:64] + bias_a
            b1 = t[64:192]
            b2 = jnp.concatenate([t[192:256], t[256:KR] + bias_d], axis=0)
            mx2 = segmax(b0, b1, b2, j)
            out.append((ha, hb, (a0, a1, a2), mx1, (b0, b1, b2), mx2))
        return out

    res = {}

    def softmax_num(segs, mx, j):
        p0 = jnp.exp2(segs[0] - jnp.where(j >= 2, mx, -NEG))
        p1 = jnp.exp2(segs[1] - jnp.where(j >= 1, mx, -NEG))
        p2 = jnp.exp2(segs[2] - mx)
        l = jnp.sum(tree(jnp.add, p0) + tree(jnp.add, p1) + tree(jnp.add, p2), axis=0, keepdims=True)
        return jnp.concatenate([p0, p1, p2], axis=0), l

    def stage_b(s, items):
        j = i * NSUB + s
        for (ha, hb, sa, mx1, sb, mx2) in items:
            p1, l1 = softmax_num(sa, mx1, j)
            p2, l2 = softmax_num(sb, mx2, j)
            pa = jnp.concatenate([jnp.where(lo64, p1[0:64], 0.0),
                                  jnp.where(lo256, p1[64:KR], p2[0:256]),
                                  jnp.where(lo64, 0.0, p2[256:KR])], axis=0).astype(jnp.bfloat16)
            pb = jnp.concatenate([jnp.where(lo64, 0.0, p1[0:64]),
                                  jnp.where(lo256, p2[0:256], p1[64:KR]),
                                  jnp.where(lo64, p2[256:KR], 0.0)], axis=0).astype(jnp.bfloat16)
            la = jnp.where(lo1, l1, l2)
            lb = jnp.where(lo1, l2, l1)
            for (h, pp, l) in ((ha, pa, la), (hb, pb, lb)):
                r0 = 80 * (h // 4) + 16 * (h % 4)
                vt = jnp.concatenate(
                    [vT_scr[j + t, r0:r0 + 32, :] for t in range(3)], axis=1)
                oh = jnp.dot(vt, pp, preferred_element_type=jnp.float32) * (1.0 / l)
                res[(s, h)] = oh if h == ha else pltpu.roll(oh, 64, 1)

    hs = {}
    bs = {}
    aa = {}

    def ffn1(s, n):
        hh = jnp.dot(x[s * 128:(s + 1) * 128], w1_ref[:, n * 512:(n + 1) * 512],
                     preferred_element_type=jnp.float32)
        hh = 0.5 * hh
        hs[(s, n)] = (hh * (1.0 + jnp.tanh(hh))).astype(jnp.bfloat16)

    def ffn2(s, m):
        hcat = jnp.concatenate([hs[(s, n)] for n in range(3)], axis=1)
        bs[(s, m)] = jnp.dot(hcat, w2_ref[:, m * 128:(m + 1) * 128], preferred_element_type=jnp.float32)

    def oproj(s):
        groups = []
        for g in range(H // 4):
            h0, h1, h2, h3 = [res[(s, 4 * g + t)] for t in range(4)]
            groups.append(jnp.concatenate([
                h0[0:16],
                jnp.where(row8 < 4, h0[16:24], h1[0:8]),
                h1[8:24],
                h2[8:24],
                jnp.where(row8 < 4, h2[24:32], h3[8:16]),
                h3[16:32],
            ], axis=0))
        oT = jnp.concatenate(groups, axis=0)
        o = oT.T.astype(jnp.bfloat16)
        aa[s] = jnp.dot(o, wo_ref[...], preferred_element_type=jnp.float32)

    def finish(s):
        z = z_scr[pl.ds(pl.multiple_of(i * TQ + s * 128, 128), 128), :][:, GLANE:GLANE + 1]
        gt = jax.nn.sigmoid(z)
        b = jnp.concatenate([bs[(s, m)] for m in range(5)], axis=1)
        o_ref[s * 128:(s + 1) * 128, :] = (gt * aa[s] + (1.0 - gt) * b).astype(o_ref.dtype)

    P = functools.partial
    f2 = lambda s, m: P(ffn2, s, m)
    f1 = lambda s, n: P(ffn1, s, n)
    sched = []
    for s in range(NSUB):
        prev = [[P(oproj, s - 1)], [P(finish, s - 1)]] if s > 0 else [[], []]
        if s < NSUB - 1:
            sched += [[f1(s, 0)], prev[0], [f1(s, 1)], prev[1], [f1(s, 2)], [],
                      [f2(s, 0)], [f2(s, 1)], [f2(s, 2)], [f2(s, 3)], [f2(s, 4)], []]
        else:
            sched += [[f1(s, 0)], prev[0], [f1(s, 1)], prev[1], [], [f1(s, 2)],
                      [], [f2(s, 0)], [], [f2(s, 1)], [f2(s, 2)], [f2(s, 3)]]
    tail = [f2(3, 4), P(oproj, 3), P(finish, 3)]

    stages = [(s, c) for s in range(NSUB) for c in range(NCH)]
    nxt = stage_a(*stages[0])
    for si, (s, c) in enumerate(stages):
        cur = nxt
        for f in sched[2 * si]:
            f()
        if si + 1 < len(stages):
            nxt = stage_a(*stages[si + 1])
        stage_b(s, cur[:1])
        for f in sched[2 * si + 1]:
            f()
        stage_b(s, cur[1:])
    for f in tail:
        f()


@jax.jit
def pallas_gated_mix__sliding_block__dense_activation_silu__prompt_kernel(
    A_x, A_wqkv, A_wo, B_x, B_w1, B_w2, gate_w):
    x = A_x.reshape(S, D)
    out = pl.pallas_call(
        _kernel,
        grid=(NST,),
        in_specs=[
            pl.BlockSpec(memory_space=pl.ANY),
            pl.BlockSpec(memory_space=pl.ANY),
            pl.BlockSpec(memory_space=pl.ANY),
            pl.BlockSpec(memory_space=pl.ANY),
            pl.BlockSpec(memory_space=pl.ANY),
            pl.BlockSpec((D,), lambda i: (0,)),
        ],
        out_specs=pl.BlockSpec((TQ, D), lambda i: (i, 0)),
        out_shape=jax.ShapeDtypeStruct((S, D), jnp.bfloat16),
        scratch_shapes=[
            pltpu.VMEM((S, D), jnp.bfloat16),
            pltpu.VMEM((S, 128), jnp.float32),
            pltpu.VMEM((D, D), jnp.bfloat16),
            pltpu.VMEM((D, DK), jnp.bfloat16),
            pltpu.VMEM((S + WIN, DK), jnp.bfloat16),
            pltpu.VMEM((NB, D, 128), jnp.float32),
            pltpu.VMEM((NB + 2, D, 128), jnp.bfloat16),
            pltpu.VMEM((2, D, D), jnp.bfloat16),
            pltpu.VMEM((D, D), jnp.bfloat16),
            pltpu.VMEM((D, F), jnp.bfloat16),
            pltpu.VMEM((F, D), jnp.bfloat16),
            pltpu.SemaphoreType.DMA((6 + NST,)),
        ],
        compiler_params=pltpu.CompilerParams(
            dimension_semantics=("arbitrary",),
            vmem_limit_bytes=100 * 2 ** 20),
    )(x, A_wqkv, A_wo, B_w1, B_w2, gate_w)
    return out.reshape(1, S, D)
```

```python
import functools
import jax
import jax.numpy as jnp
import jax.experimental.pallas as pl
import jax.experimental.pallas.tpu as pltpu

S, D, H, DH, WIN, F = 2048, 640, 32, 20, 256, 1536
TQ = 512
NSUB = TQ // 128
NST = S // TQ
NB = S // 128
NT = (((1,), (1,)), ((), ()))
LOG2E = 1.4426950408889634
NEG = -1e9

XOFF = {6: 0, 19: 20, 12: 40, 25: 60, 8: 80, 21: 100}
CH = [[(h, 128 * c, DH * h - 128 * c) for h in range(H)
       if (DH * h) // 128 == c and h not in XOFF] for c in range(5)]
CH.append([(h, DH * h - XOFF[h], XOFF[h]) for h in XOFF])
NCH = len(CH)
DK = 128 * NCH
KR = WIN + 64


def _kernel(x_hbm, wqkv_hbm, wo_hbm, w1_hbm, w2_hbm, gw_ref, o_ref,
            x_scr, z_scr, wT_scr, wk_scr, k_scr, qT_scr, vT_scr, wqv_ref, wo_ref, w1_ref, w2_ref, sems):
    i = pl.program_id(0)

    @pl.when(i == 0)
    def _():
        cp_x = [pltpu.make_async_copy(x_hbm.at[b * TQ:(b + 1) * TQ, :], x_scr.at[b * TQ:(b + 1) * TQ, :],
                                      sems.at[6 + b]) for b in range(NST)]
        cp_q = pltpu.make_async_copy(wqkv_hbm.at[:, 0:D], wqv_ref.at[0], sems.at[0])
        cp_k = pltpu.make_async_copy(wqkv_hbm.at[:, D:2 * D], wk_scr, sems.at[1])
        cp_v = pltpu.make_async_copy(wqkv_hbm.at[:, 2 * D:3 * D], wqv_ref.at[1], sems.at[2])
        cp_w1 = pltpu.make_async_copy(w1_hbm, w1_ref, sems.at[3])
        cp_w2 = pltpu.make_async_copy(w2_hbm, w2_ref, sems.at[4])
        cp_wo = pltpu.make_async_copy(wo_hbm, wo_ref, sems.at[5])
        cp_k.start()
        cp_x[0].start()
        cp_x[1].start()
        cp_q.start()
        cp_x[2].start()
        cp_x[3].start()
        cp_v.start()
        cp_w1.start()
        cp_w2.start()
        cp_wo.start()
        k_scr[0:WIN, :] = jnp.zeros((WIN, DK), jnp.bfloat16)
        vT_scr[0:2] = jnp.zeros((2, D, 128), jnp.bfloat16)
        cp_k.wait()
        lane = jax.lax.broadcasted_iota(jnp.int32, (TQ, 128), 1)

        def xblk(b):
            return x_scr[pl.ds(pl.multiple_of(b * TQ, TQ), TQ), :]

        def kproj(b, carry):
            rows = pl.ds(pl.multiple_of(b * TQ, TQ), TQ)
            pltpu.make_async_copy(x_hbm.at[rows, :], x_scr.at[rows, :], sems.at[6 + b]).wait()
            xb = xblk(b)
            k = jnp.dot(xb, wk_scr[...], preferred_element_type=jnp.float32)
            krows = pl.ds(pl.multiple_of(WIN + b * TQ, 128), TQ)
            k_scr[krows, 0:D] = k.astype(jnp.bfloat16)
            z = jnp.sum(xb.astype(jnp.float32) * gw_ref[...].astype(jnp.float32).reshape(1, D),
                        axis=-1, keepdims=True)
            z_scr[rows, :] = jnp.broadcast_to(jax.nn.sigmoid(z), (TQ, 128))
            return carry
        jax.lax.fori_loop(0, NST - 1, kproj, 0)
        cp_q.wait()
        kproj(NST - 1, 0)
        wT_scr[...] = wqv_ref[0].T

        def kextra(b):
            krows = pl.ds(pl.multiple_of(WIN + b * TQ, 128), TQ)
            k = k_scr[krows, 0:D].astype(jnp.float32)
            kx = None
            for h in XOFF:
                c0, lo = (DH * h) // 128, (DH * h) % 128
                y = k[:, c0 * 128:(c0 + 1) * 128]
                if lo + DH > 128:
                    y = jnp.where(lane >= lo, y, k[:, (c0 + 1) * 128:(c0 + 2) * 128])
                y = pltpu.roll(y, (XOFF[h] - lo) % 128, 1)
                kx = y if kx is None else jnp.where(lane >= XOFF[h], y, kx)
            k_scr[krows, D:DK] = kx.astype(jnp.bfloat16)

        def qproj(b, carry):
            kextra(b)
            qT = jax.lax.dot_general(wT_scr[...], xblk(b), NT, preferred_element_type=jnp.float32)
            qT = qT * (DH ** -0.5 * LOG2E)
            for s in range(NSUB):
                qT_scr[b * NSUB + s] = qT[:, s * 128:(s + 1) * 128]
            return carry
        jax.lax.fori_loop(0, NST - 1, qproj, 0)
        cp_v.wait()
        qproj(NST - 1, 0)
        wqv_ref[0] = wqv_ref[1].T

        def vproj(b, carry):
            vT = jax.lax.dot_general(wqv_ref[0], xblk(b), NT,
                                     preferred_element_type=jnp.float32).astype(jnp.bfloat16)
            for s in range(NSUB):
                vT_scr[2 + b * NSUB + s] = vT[:, s * 128:(s + 1) * 128]
            return carry
        jax.lax.fori_loop(0, NST, vproj, 0)
        cp_w1.wait()
        cp_w2.wait()
        cp_wo.wait()

    x = x_scr[pl.ds(pl.multiple_of(i * TQ, TQ), TQ), :]

    row128 = jax.lax.broadcasted_iota(jnp.int32, (128, 128), 0)
    lo128 = jax.lax.broadcasted_iota(jnp.int32, (128, 128), 1) < 64
    row8 = jax.lax.broadcasted_iota(jnp.int32, (8, 128), 0)
    r64 = jax.lax.broadcasted_iota(jnp.int32, (64, 128), 0)
    c64 = jax.lax.broadcasted_iota(jnp.int32, (64, 128), 1) & 63
    bias_a = jnp.where(r64 > c64, 0.0, NEG)
    bias_d = jnp.where(r64 <= c64, 0.0, NEG)
    lo1 = jax.lax.broadcasted_iota(jnp.int32, (1, 128), 1) < 64
    lo64 = jax.lax.broadcasted_iota(jnp.int32, (64, 128), 1) < 64
    lo256 = jax.lax.broadcasted_iota(jnp.int32, (256, 128), 1) < 64

    def tree(op, v):
        n = v.shape[0]
        while n > 8:
            h = n // 2
            v = op(v[0:h], v[h:n])
            n = h
        return v

    def segmax(v0, v1, v2, j):
        m = jnp.maximum(jnp.maximum(jnp.where(j >= 2, tree(jnp.maximum, v0), NEG),
                                    jnp.where(j >= 1, tree(jnp.maximum, v1), NEG)),
                        tree(jnp.maximum, v2))
        return jnp.max(m, axis=0, keepdims=True)

    def stage_a(s, c):
        j = i * NSUB + s
        koff = pl.multiple_of(j * 128, 128)
        w1s, w2s = [], []
        heads = CH[c]
        for p in range(len(heads) // 2):
            (ha, ra, oa), (hb, rb, ob) = heads[2 * p], heads[2 * p + 1]
            qa = qT_scr[j, ra:ra + 128, :]
            qa = jnp.where((row128 >= oa) & (row128 < oa + DH), qa, 0.0)
            qb = qT_scr[j, rb:rb + 128, :]
            qb = jnp.where((row128 >= ob) & (row128 < ob + DH), qb, 0.0)
            qbr = pltpu.roll(qb, 64, 1)
            w1s.append(jnp.where(lo128, qa, qbr).astype(jnp.bfloat16))
            w2s.append(jnp.where(lo128, qbr, qa).astype(jnp.bfloat16))
        k1 = k_scr[pl.ds(koff, KR), c * 128:(c + 1) * 128]
        k2 = k_scr[pl.ds(koff + 64, KR), c * 128:(c + 1) * 128]
        s1all = jnp.dot(k1, jnp.concatenate(w1s, axis=1), preferred_element_type=jnp.float32)
        s2all = jnp.dot(k2, jnp.concatenate(w2s, axis=1), preferred_element_type=jnp.float32)
        out = []
        for p in range(len(heads) // 2):
            ha, hb = heads[2 * p][0], heads[2 * p + 1][0]
            t = s1all[:, p * 128:(p + 1) * 128]
            a0 = jnp.concatenate([t[0:64] + bias_a, t[64:128]], axis=0)
            a1 = t[128:256]
            a2 = t[256:KR] + bias_d
            mx1 = segmax(a0, a1, a2, j)
            t = s2all[:, p * 128:(p + 1) * 128]
            b0 = t[0:64] + bias_a
            b1 = t[64:192]
            b2 = jnp.concatenate([t[192:256], t[256:KR] + bias_d], axis=0)
            mx2 = segmax(b0, b1, b2, j)
            out.append((ha, hb, (a0, a1, a2), mx1, (b0, b1, b2), mx2))
        return out

    res = {}

    def softmax_num(segs, mx, j):
        p0 = jnp.exp2(segs[0] - jnp.where(j >= 2, mx, -NEG))
        p1 = jnp.exp2(segs[1] - jnp.where(j >= 1, mx, -NEG))
        p2 = jnp.exp2(segs[2] - mx)
        l = jnp.sum(tree(jnp.add, p0) + tree(jnp.add, p1) + tree(jnp.add, p2), axis=0, keepdims=True)
        return jnp.concatenate([p0, p1, p2], axis=0), l

    def stage_b(s, items):
        j = i * NSUB + s
        for (ha, hb, sa, mx1, sb, mx2) in items:
            p1, l1 = softmax_num(sa, mx1, j)
            p2, l2 = softmax_num(sb, mx2, j)
            pa = jnp.concatenate([jnp.where(lo64, p1[0:64], 0.0),
                                  jnp.where(lo256, p1[64:KR], p2[0:256]),
                                  jnp.where(lo64, 0.0, p2[256:KR])], axis=0).astype(jnp.bfloat16)
            pb = jnp.concatenate([jnp.where(lo64, 0.0, p1[0:64]),
                                  jnp.where(lo256, p2[0:256], p1[64:KR]),
                                  jnp.where(lo64, p2[256:KR], 0.0)], axis=0).astype(jnp.bfloat16)
            la = jnp.where(lo1, l1, l2)
            lb = jnp.where(lo1, l2, l1)
            for (h, pp, l) in ((ha, pa, la), (hb, pb, lb)):
                r0 = 80 * (h // 4) + 16 * (h % 4)
                vt = jnp.concatenate(
                    [vT_scr[j + t, r0:r0 + 32, :] for t in range(3)], axis=1)
                oh = jnp.dot(vt, pp, preferred_element_type=jnp.float32) * (1.0 / l)
                res[(s, h)] = oh if h == ha else pltpu.roll(oh, 64, 1)

    hs = {}
    bs = {}
    aa = {}

    def ffn1(s, n):
        hh = jnp.dot(x[s * 128:(s + 1) * 128], w1_ref[:, n * 512:(n + 1) * 512],
                     preferred_element_type=jnp.float32)
        hh = 0.5 * hh
        hs[(s, n)] = (hh * (1.0 + jnp.tanh(hh))).astype(jnp.bfloat16)

    def ffn2(s, m):
        hcat = jnp.concatenate([hs[(s, n)] for n in range(3)], axis=1)
        bs[(s, m)] = jnp.dot(hcat, w2_ref[:, m * 128:(m + 1) * 128], preferred_element_type=jnp.float32)

    def oproj(s):
        groups = []
        for g in range(H // 4):
            h0, h1, h2, h3 = [res[(s, 4 * g + t)] for t in range(4)]
            groups.append(jnp.concatenate([
                h0[0:16],
                jnp.where(row8 < 4, h0[16:24], h1[0:8]),
                h1[8:24],
                h2[8:24],
                jnp.where(row8 < 4, h2[24:32], h3[8:16]),
                h3[16:32],
            ], axis=0))
        oT = jnp.concatenate(groups, axis=0)
        o = oT.T.astype(jnp.bfloat16)
        aa[s] = jnp.dot(o, wo_ref[...], preferred_element_type=jnp.float32)

    def finish(s):
        g = z_scr[pl.ds(pl.multiple_of(i * TQ + s * 128, 128), 128), :]
        gt = jnp.concatenate([g] * 5, axis=1)
        b = jnp.concatenate([bs[(s, m)] for m in range(5)], axis=1)
        o_ref[s * 128:(s + 1) * 128, :] = (gt * aa[s] + (1.0 - gt) * b).astype(o_ref.dtype)

    P = functools.partial
    f2 = lambda s, m: P(ffn2, s, m)
    f1 = lambda s, n: P(ffn1, s, n)
    sched = []
    for s in range(NSUB):
        prev = [[P(oproj, s - 1)], [P(finish, s - 1)]] if s > 0 else [[], []]
        if s < NSUB - 1:
            sched += [[f1(s, 0)], prev[0], [f1(s, 1)], prev[1], [f1(s, 2)], [],
                      [f2(s, 0)], [f2(s, 1)], [f2(s, 2)], [f2(s, 3)], [f2(s, 4)], []]
        else:
            sched += [[f1(s, 0)], prev[0], [f1(s, 1)], prev[1], [f1(s, 2)], [f2(s, 0)],
                      [], [f2(s, 1)], [], [f2(s, 2)], [], [f2(s, 3)]]
    tail = [f2(NSUB - 1, 4), P(oproj, NSUB - 1), P(finish, NSUB - 1)]

    stages = [(s, c) for s in range(NSUB) for c in range(NCH)]
    nxt = stage_a(*stages[0])
    for si, (s, c) in enumerate(stages):
        cur = nxt
        for f in sched[2 * si]:
            f()
        if si + 1 < len(stages):
            nxt = stage_a(*stages[si + 1])
        stage_b(s, cur[:1])
        for f in sched[2 * si + 1]:
            f()
        stage_b(s, cur[1:])
    for f in tail:
        f()


@jax.jit
def pallas_gated_mix__sliding_block__dense_activation_silu__prompt_kernel(
    A_x: jax.Array,
    A_wqkv: jax.Array,
    A_wo: jax.Array,
    B_x: jax.Array,
    B_w1: jax.Array,
    B_w2: jax.Array,
    gate_w: jax.Array,
):
    del B_x
    x = A_x.reshape(S, D)
    out = pl.pallas_call(
        _kernel,
        grid=(NST,),
        in_specs=[
            pl.BlockSpec(memory_space=pl.ANY),
            pl.BlockSpec(memory_space=pl.ANY),
            pl.BlockSpec(memory_space=pl.ANY),
            pl.BlockSpec(memory_space=pl.ANY),
            pl.BlockSpec(memory_space=pl.ANY),
            pl.BlockSpec((D,), lambda i: (0,)),
        ],
        out_specs=pl.BlockSpec((TQ, D), lambda i: (i, 0)),
        out_shape=jax.ShapeDtypeStruct((S, D), jnp.bfloat16),
        scratch_shapes=[
            pltpu.VMEM((S, D), jnp.bfloat16),
            pltpu.VMEM((S, 128), jnp.float32),
            pltpu.VMEM((D, D), jnp.bfloat16),
            pltpu.VMEM((D, D), jnp.bfloat16),
            pltpu.VMEM((S + WIN, DK), jnp.bfloat16),
            pltpu.VMEM((NB, D, 128), jnp.float32),
            pltpu.VMEM((NB + 2, D, 128), jnp.bfloat16),
            pltpu.VMEM((2, D, D), jnp.bfloat16),
            pltpu.VMEM((D, D), jnp.bfloat16),
            pltpu.VMEM((D, F), jnp.bfloat16),
            pltpu.VMEM((F, D), jnp.bfloat16),
            pltpu.SemaphoreType.DMA((6 + NST,)),
        ],
        compiler_params=pltpu.CompilerParams(
            dimension_semantics=("arbitrary",),
            vmem_limit_bytes=100 * 2 ** 20),
    )(x, A_wqkv, A_wo, B_w1, B_w2, gate_w)
    return out.reshape(1, S, D)
```
